```python
import os as _os
_os.environ.setdefault("JAX_PLATFORMS", "cpu")
import jax
import jax.numpy as jnp

def _softmax(x, axis=-1):
    return jax.nn.softmax(x, axis=axis)
def _gelu(x):
    return jax.nn.gelu(x, approximate=True)
def _silu(x):
    return jax.nn.silu(x)
def _sigmoid(x):
    return jax.nn.sigmoid(x)
def _layernorm(x, axis=-1, eps=1e-5):
    m = jnp.mean(x, axis=axis, keepdims=True)
    v = jnp.var(x, axis=axis, keepdims=True)
    return (x - m) / jnp.sqrt(v + eps)
def _scatter_add(tgt, idx, src, axis=0):
    return tgt.at[idx].add(src)
def _segment_sum(src, seg, n):
    return jax.ops.segment_sum(src, seg, n)
class _Rng:
    def __init__(self, key):
        self._k = key
    def _next(self):
        self._k, sub = jax.random.split(self._k)
        return sub
    def normal(self, shape):
        return jax.random.normal(self._next(), shape, dtype=jnp.bfloat16)
    def randint(self, lo, hi, shape):
        return jax.random.randint(self._next(), shape, lo, hi, dtype=jnp.int32)
    def uniform(self, shape, lo=0.0, hi=1.0):
        return jax.random.uniform(self._next(), shape, jnp.bfloat16, lo, hi)
    def permutation(self, n):
        return jax.random.permutation(self._next(), n)


kernel_name = 'standalone__se_block__vision'

def setup_inputs():
    _rng = _Rng(jax.random.key(int.from_bytes(__import__("os").urandom(4), "little")))
    _w = (lambda a: (lambda t: t.astype(jnp.bfloat16) if jnp.issubdtype(t.dtype, jnp.floating) else t)(jnp.asarray(a)))
    H = W = 384
    C = 192; r = max(C // 16, 4)
    return {
        "x": _w((lambda *s: _rng.normal(s) * 0.8)(1, H, W, C)),
        "w_down": _w((lambda *s: _rng.normal(s) * 0.8)(C, r)),
        "w_up": _w((lambda *s: _rng.normal(s) * 0.8)(r, C)),
    }

def reference(x, w_down, w_up):
    s = x.mean(axis=(1, 2))
    s = _sigmoid(_silu(s @ w_down) @ w_up)
    return x * s[:, None, None, :]
```

```python
import functools
import jax
import jax.numpy as jnp
from jax import lax
import jax.experimental.pallas as pl
import jax.experimental.pallas.tpu as pltpu

A1, A0, NJ, PR, LN = 12, 9, 32, 64, 128


def make(inflight=4, in_tail=(6, 3, 2, 1), out_head=(1, 2, 3, 6), vmem_mb=100):
    def kernel(x_hbm, wdt_hbm, wu_hbm, o_hbm, buf, acc, scale, wdt_v, wu_v, sem_in, sem_tail, sem_w, sem_out, sem_head):
        def cin(j):
            return pltpu.make_async_copy(x_hbm.at[:, :, j], buf.at[:, :, j], sem_in.at[j])

        def cout(j):
            return pltpu.make_async_copy(buf.at[:, :, j], o_hbm.at[:, :, j], sem_out.at[j])

        tail_off = [sum(in_tail[:i]) for i in range(len(in_tail))]
        head_off = [sum(out_head[:i]) for i in range(len(out_head))]

        def cin_tail(i):
            return pltpu.make_async_copy(
                x_hbm.at[pl.ds(tail_off[i], in_tail[i]), :, NJ - 1],
                buf.at[pl.ds(tail_off[i], in_tail[i]), :, NJ - 1], sem_tail.at[i])

        def cout_head(i):
            return pltpu.make_async_copy(
                buf.at[pl.ds(head_off[i], out_head[i]), :, 0],
                o_hbm.at[pl.ds(head_off[i], out_head[i]), :, 0], sem_head.at[i])

        NM = NJ - 1
        for j in range(NM):
            cin(j).start()
        for i in range(len(in_tail)):
            cin_tail(i).start()
        cw0 = pltpu.make_async_copy(wdt_hbm, wdt_v, sem_w.at[0])
        cw1 = pltpu.make_async_copy(wu_hbm, wu_v, sem_w.at[1])
        cw0.start(priority=1)
        cw1.start(priority=1)

        acc[...] = jnp.zeros(acc.shape, jnp.float32)

        def accum(lo, n, a0, j):
            blk = lax.rem(5 * a0 + j, A0)
            v = buf[pl.ds(lo, n), a0, j].astype(jnp.float32)
            acc[blk] += jnp.sum(v, axis=0)

        def in_body(j, carry):
            cin(j).wait()
            def inner(a0, c):
                accum(0, A1, a0, j)
                return c
            lax.fori_loop(0, A0, inner, 0)
            return carry
        lax.fori_loop(0, NM, in_body, 0)

        cw0.wait()
        cw1.wait()
        wdt = wdt_v[...]
        wut = wu_v[...].astype(jnp.float32).T.astype(jnp.bfloat16)

        for i in range(len(in_tail)):
            cin_tail(i).wait()
            for a0 in range(A0):
                blk = (5 * a0 + NJ - 1) % A0
                v = buf[pl.ds(tail_off[i], in_tail[i]), a0, NJ - 1].astype(jnp.float32)
                acc[blk] += jnp.sum(v, axis=0)

        tot = acc[...].reshape(24, 3, 8, LN).sum(axis=1).reshape(192, LN)
        mean = jnp.sum(tot, axis=1, keepdims=True) * (1.0 / (384 * 384))
        mean_b = jnp.broadcast_to(mean, (192, LN)).astype(jnp.bfloat16)
        h = jnp.dot(wdt, mean_b, preferred_element_type=jnp.float32)
        h = h.astype(jnp.bfloat16).astype(jnp.float32)
        h = (h * jax.nn.sigmoid(h)).astype(jnp.bfloat16)
        g = jnp.dot(wut, h, preferred_element_type=jnp.float32)
        g = g.astype(jnp.bfloat16).astype(jnp.float32)
        s = jax.nn.sigmoid(g).astype(jnp.bfloat16).astype(jnp.float32)
        s3 = jnp.broadcast_to(s.reshape(24, 1, 8, LN), (24, 3, 8, LN)).reshape(A0, PR, LN)
        scale[...] = s3

        for i in range(len(out_head)):
            for a0 in range(A0):
                blk = (5 * a0) % A0
                sl = (pl.ds(head_off[i], out_head[i]), a0, 0)
                buf[sl] = (buf[sl].astype(jnp.float32) * scale[blk][None]).astype(jnp.bfloat16)
            cout_head(i).start()

        def out_body(j, carry):
            def inner(a0, c):
                blk = lax.rem(5 * a0 + j, A0)
                sl = (slice(None), a0, j)
                buf[sl] = (buf[sl].astype(jnp.float32) * scale[blk][None]).astype(jnp.bfloat16)
                return c
            lax.fori_loop(0, A0, inner, 0)
            cout(j).start()
            return carry
        lax.fori_loop(1, NJ, out_body, 0)

        for i in range(len(out_head)):
            cout_head(i).wait()
        def wait_body(j, carry):
            cout(j).wait()
            return carry
        lax.fori_loop(1, NJ, wait_body, 0)

    @jax.jit
    def f(x, w_down, w_up):
        _, H, W, C = x.shape
        xt = jnp.transpose(x, (0, 1, 3, 2)).reshape(H, C // 8, 8, W // LN, LN)
        xt = jnp.transpose(xt, (0, 1, 3, 2, 4)).reshape(A1, A0, NJ, PR, LN)
        o = pl.pallas_call(
            kernel,
            out_shape=jax.ShapeDtypeStruct((A1, A0, NJ, PR, LN), x.dtype),
            in_specs=[pl.BlockSpec(memory_space=pl.ANY)] * 3,
            out_specs=pl.BlockSpec(memory_space=pl.ANY),
            scratch_shapes=[
                pltpu.VMEM((A1, A0, NJ, PR, LN), x.dtype),
                pltpu.VMEM((A0, PR, LN), jnp.float32),
                pltpu.VMEM((A0, PR, LN), jnp.float32),
                pltpu.VMEM((12, 192), x.dtype),
                pltpu.VMEM((12, 192), x.dtype),
                pltpu.SemaphoreType.DMA((NJ,)),
                pltpu.SemaphoreType.DMA((len(in_tail),)),
                pltpu.SemaphoreType.DMA((2,)),
                pltpu.SemaphoreType.DMA((NJ,)),
                pltpu.SemaphoreType.DMA((len(out_head),)),
            ],
            compiler_params=pltpu.CompilerParams(vmem_limit_bytes=vmem_mb * 1024 * 1024),
        )(xt, w_down.T, w_up)
        o = o.reshape(H, C // 8, W // LN, 8, LN)
        o = jnp.transpose(o, (0, 1, 3, 2, 4)).reshape(1, H, C, W)
        return jnp.transpose(o, (0, 1, 3, 2))
    return f


pallas_standalone__se_block__vision_kernel = make()
```

```python
import jax
import jax.numpy as jnp
from jax import lax
import jax.experimental.pallas as pl
import jax.experimental.pallas.tpu as pltpu

F32 = jnp.float32

H, W, C, R = 384, 384, 192, 12
LN = 128
RH = C * W // LN
NG = C // 8

NH = 8
NSEM = 4
CN = C - 16
RC = 3 * CN
TAIL_EARLY = (8, 8, 4, 4)
TAIL_LATE = (18, 4, 2)
NMAIN = (H - sum(TAIL_EARLY)) // NH

G, A, RS = 9, 6, 4096
P0, P = 64, 48
NP = (RS - P0) // P
NSTATIC = 2
NTAB = 16


def _tails():
    out = []
    for sizes, r0, nr in ((TAIL_EARLY, 0, RC), (TAIL_LATE, RC, RH - RC)):
        h0 = NMAIN * NH
        for n in sizes:
            out.append((h0, n, r0, nr))
            h0 += n
        assert h0 == H
    return out


TAILS = _tails()


def _tree_sum(terms):
    while len(terms) > 1:
        terms = [terms[i] + terms[i + 1] if i + 1 < len(terms) else terms[i]
                 for i in range(0, len(terms), 2)]
    return terms[0]


def _body(x_hbm, wdt_hbm, wu_hbm, o_hbm, buf, acc, stab, wdt_v, wu_v, wdc, wub, sem_x, sem_in):
    def read(i):
        if isinstance(i, int):
            h0, slot = i * NH, i % NSEM
        else:
            h0, slot = pl.multiple_of(i * NH, NH), lax.rem(i, NSEM)
        return pltpu.make_async_copy(
            x_hbm.at[pl.ds(h0, NH)], buf.at[pl.ds(h0, NH)], sem_in.at[slot])

    def read_tail(t):
        h0, n, r0, nr = TAILS[t]
        return pltpu.make_async_copy(
            x_hbm.at[pl.ds(h0, n), pl.ds(r0, nr)], buf.at[pl.ds(h0, n), pl.ds(r0, nr)],
            sem_in.at[(NMAIN + t) % NSEM])

    read(0).start()
    w_copies = [pltpu.make_async_copy(wdt_hbm, wdt_v, sem_x),
                pltpu.make_async_copy(wu_hbm, wu_v, sem_x)]
    for cp in w_copies:
        cp.start()
    for i in range(1, NSEM):
        read(i).start()

    acc[...] = jnp.zeros(acc.shape, F32)

    for cp in w_copies:
        cp.wait()
    down_scale = 0.5 / (H * W)
    wdt = wdt_v[...].astype(F32) * down_scale
    for c in range(C - CN):
        wdc[c] = jnp.broadcast_to(wdt[:, CN + c:CN + c + 1], (R, LN))
    wut = wu_v[...].astype(F32).T * 0.5
    for k in range(R):
        wub[k] = jnp.broadcast_to(wut[:, k:k + 1], (C, LN))

    def pair_sum(h0, n, q):
        v = jnp.sum(buf[pl.ds(h0, n), pl.ds(48 * q, 48)].astype(F32), axis=0)
        return jnp.concatenate(
            [v[0:8] + v[8:16] + v[16:24], v[24:32] + v[32:40] + v[40:48]], axis=0)

    def accumulate(h0, n, nq):
        for q in range(nq):
            acc[pl.ds(16 * q, 16)] += pair_sum(h0, n, q)

    def main_step(i, carry):
        read(i).wait()
        read(i + NSEM).start()
        accumulate(pl.multiple_of(i * NH, NH), NH, NG // 2)
        return carry

    def drain_step(i, carry):
        read(i).wait()
        for t in range(NSEM):
            pl.when(i == NMAIN - NSEM + t)(read_tail(t).start)
        accumulate(pl.multiple_of(i * NH, NH), NH, NG // 2)
        return carry

    lax.fori_loop(0, NMAIN - NSEM, main_step, 0)
    lax.fori_loop(NMAIN - NSEM, NMAIN, drain_step, 0)

    def wait_tail(t):
        read_tail(t).wait()
        if t + NSEM < len(TAILS):
            read_tail(t + NSEM).start()

    for t in range(len(TAIL_EARLY)):
        wait_tail(t)
        accumulate(TAILS[t][0], TAILS[t][1], CN // 16)

    sums = jnp.broadcast_to(jnp.sum(acc[pl.ds(0, CN)], axis=1, keepdims=True), (CN, LN))
    wdc[C - CN] = jnp.dot(wdt_v[:, pl.ds(0, CN)].astype(F32) * down_scale, sums,
                          preferred_element_type=F32, precision=lax.Precision.HIGHEST)
    late = acc[pl.ds(CN, C - CN)]
    for t in range(len(TAIL_EARLY), len(TAILS)):
        wait_tail(t)
        late = late + pair_sum(TAILS[t][0], TAILS[t][1], CN // 16)
    late = jnp.broadcast_to(jnp.sum(late, axis=1, keepdims=True), (C - CN, LN))
    p = _tree_sum([wdc[C - CN]] + [wdc[c] * late[c:c + 1] for c in range(C - CN)])
    hid = p * jnp.tanh(p) + p
    hid = [jnp.broadcast_to(hid[k:k + 1], (8, LN)) for k in range(R)]

    gates = {}

    def gate(g):
        if g not in gates:
            z = _tree_sum([wub[k, pl.ds(8 * g, 8)] * hid[k] for k in range(R)])
            gates[g] = 0.5 * jnp.tanh(z) + 0.5
        return gates[g]

    ov = buf.reshape(G, A, RS, LN)

    def rows(get, tile0, nrows):
        return jnp.concatenate([get((tile0 + i) // 3) for i in range(nrows // 8)], axis=0)

    def stripes(get, tile0, nrows):
        return jnp.stack([rows(get, tile0 + 8 * a, nrows) for a in range(A)])

    def emit(sl, scale):
        ov[sl] = (ov[sl].astype(F32) * scale).astype(ov.dtype)
        pltpu.make_async_copy(ov.at[sl], o_hbm.at[sl], sem_x).start()

    for a in range(A):
        emit((0, a, pl.ds(0, P0)), rows(gate, 8 * a, P0))
    for i in range(NSTATIC):
        emit((0, slice(None), pl.ds(P0 + P * i, P)), stripes(gate, (P0 + P * i) // 8, P))
    for g in range(stab.shape[0]):
        stab[g] = gate(g % NG)

    def piece(g, i, u):
        tab = stab[pl.ds(u, NTAB)]
        r0 = pl.multiple_of(P0 + P * i, 16)
        emit((g, slice(None), pl.ds(r0, P)), stripes(lambda q: tab[q], 2, P))
        return jnp.where(u == NG - 2, 0, u + 2)

    def group(g, u0):
        tab = stab[pl.ds(u0, NTAB)]
        emit((g, slice(None), pl.ds(0, P0)), stripes(lambda q: tab[q], 0, P0))
        lax.fori_loop(0, NP, lambda i, u: piece(g, i, u), u0 + 2)
        return jnp.where(u0 >= 8, u0 - 8, u0 + 16)

    lax.fori_loop(NSTATIC, NP, lambda i, u: piece(0, i, u), 2 + 2 * NSTATIC)
    lax.fori_loop(1, G, group, 16)


def _kernel(x_hbm, wdt_hbm, wu_hbm, o_hbm, buf, *scratch):
    def with_sem(sem_x):
        pl.run_scoped(
            lambda sem_in: _body(x_hbm, wdt_hbm, wu_hbm, o_hbm, buf, *scratch, sem_x, sem_in),
            pltpu.SemaphoreType.DMA((NSEM,)))
        pltpu.make_async_copy(buf.reshape(G, A, RS, LN), o_hbm, sem_x).wait()

    pl.run_scoped(with_sem, pltpu.SemaphoreType.DMA(()))


@jax.jit
def pallas_standalone__se_block__vision_kernel(
    x: jax.Array,
    w_down: jax.Array,
    w_up: jax.Array,
):
    assert x.shape == (1, H, W, C) and w_down.shape == (C, R) and w_up.shape == (R, C)
    xt = jnp.transpose(x, (0, 1, 3, 2)).reshape(H, NG, 8, W // LN, LN)
    xt = jnp.transpose(xt, (0, 1, 3, 2, 4)).reshape(H, RH, LN)
    out = pl.pallas_call(
        _kernel,
        out_shape=jax.ShapeDtypeStruct((G, A, RS, LN), x.dtype),
        in_specs=[pl.BlockSpec(memory_space=pl.ANY)] * 3,
        out_specs=pl.BlockSpec(memory_space=pl.ANY),
        scratch_shapes=[
            pltpu.VMEM((H, RH, LN), x.dtype),
            pltpu.VMEM((C, LN), F32),
            pltpu.VMEM((NG + NTAB - 2, 8, LN), F32),
            pltpu.VMEM((R, C), w_down.dtype),
            pltpu.VMEM((R, C), w_up.dtype),
            pltpu.VMEM((C - CN + 1, R, LN), F32),
            pltpu.VMEM((R, C, LN), F32),
        ],
        compiler_params=pltpu.CompilerParams(vmem_limit_bytes=100 * 1024 * 1024),
    )(xt, w_down.T, w_up)
    out = out.reshape(H, NG, W // LN, 8, LN)
    out = jnp.transpose(out, (0, 1, 3, 2, 4)).reshape(1, H, C, W)
    return jnp.transpose(out, (0, 1, 3, 2))
```

```python
import jax
import jax.numpy as jnp
from jax import lax
import jax.experimental.pallas as pl
import jax.experimental.pallas.tpu as pltpu

F32 = jnp.float32
LOG2E = 1.4426950408889634

H, W, C, R = 384, 384, 192, 12
LN = 128
RH = C * W // LN
NG = C // 8
NS, RS = 54, 4096
RB = 64
NB = RH // RB

NSEM = 4
CN = C - 16
RC = 3 * CN
TAIL_EARLY = (8, 8, 4, 4)
TAIL_LATE = (18, 4, 2)

G, A = 9, 6
P0, P = 64, 48
NP = (RS - P0) // P
NSTATIC = 2
NTAB = 16


def _split(row0, nrows):
    out = []
    while nrows:
        s, r = divmod(row0, RS)
        n = min(nrows, RS - r)
        out.append((s, r, n))
        row0, nrows = row0 + n, nrows - n
    return out


def _plan_reads():
    h_tail = H - sum(TAIL_EARLY)
    nmain = h_tail * RH // RS
    groups = [((), _split(nmain * RS, h_tail * RH - nmain * RS))]
    for sizes, r0, nr in ((TAIL_EARLY, 0, RC), (TAIL_LATE, RC, RH - RC)):
        h0 = h_tail
        for n in sizes:
            hs = range(h0, h0 + n)
            groups.append((hs, [p for h in hs for p in _split(h * RH + r0, nr)]))
            h0 += n
        assert h0 == H
    return nmain, groups


NMAIN, TAILS = _plan_reads()


def _tree_sum(terms):
    while len(terms) > 1:
        terms = [terms[i] + terms[i + 1] if i + 1 < len(terms) else terms[i]
                 for i in range(0, len(terms), 2)]
    return terms[0]


def _inv_1p_exp2(q):
    d = 1.0 + jnp.exp2(jnp.minimum(q, 120.0))
    r = pl.reciprocal(d, approx=True)
    return r * (2.0 - d * r)


def _body(x_hbm, wdt_hbm, wu_hbm, o_hbm, buf, accb, acc, stab, wdt_v, wu_v, wdc, wub,
          sem_x, sem_in):
    def read(s):
        slot = s % NSEM if isinstance(s, int) else lax.rem(s, NSEM)
        return pltpu.make_async_copy(x_hbm.at[s], buf.at[s], sem_in.at[slot])

    def tail_copies(t):
        return [pltpu.make_async_copy(x_hbm.at[s, pl.ds(r, n)], buf.at[s, pl.ds(r, n)],
                                      sem_in.at[(NMAIN + t) % NSEM])
                for s, r, n in TAILS[t][1]]

    def start_tail(t):
        for cp in tail_copies(t):
            cp.start()

    def wait_tail(t):
        for cp in tail_copies(t):
            cp.wait()
        if t + NSEM < len(TAILS):
            start_tail(t + NSEM)

    read(0).start()
    w_copies = [pltpu.make_async_copy(wdt_hbm, wdt_v, sem_x),
                pltpu.make_async_copy(wu_hbm, wu_v, sem_x)]
    for cp in w_copies:
        cp.start()
    for s in range(1, NSEM):
        read(s).start()

    accb[...] = jnp.zeros(accb.shape, F32)

    def add_blocks(s, b0, nblocks):
        for k in range(NB):
            v = buf[s, pl.ds(RB * k, RB)].astype(F32)
            for j in range(k + NB, nblocks, NB):
                v = v + buf[s, pl.ds(RB * j, RB)].astype(F32)
            b = b0 + k
            b = b % NB if isinstance(b, int) else jnp.where(b >= NB, b - NB, b)
            accb[b] += v

    def main_step(s, b0):
        read(s).wait()
        read(s + NSEM).start()
        add_blocks(s, b0, RS // RB)
        return jnp.where(b0 == NB - 1, 0, b0 + 1)

    def drain_step(s, b0):
        read(s).wait()
        for t in range(NSEM):
            pl.when(s == NMAIN - NSEM + t)(lambda t=t: start_tail(t))
        add_blocks(s, b0, RS // RB)
        return jnp.where(b0 == NB - 1, 0, b0 + 1)

    lax.fori_loop(0, NMAIN - NSEM, main_step, 0)

    for cp in w_copies:
        cp.wait()
    down_scale = -LOG2E / (H * W)
    wdt = wdt_v[...].astype(F32) * down_scale
    for c in range(C - CN):
        wdc[c] = jnp.broadcast_to(wdt[:, CN + c:CN + c + 1], (R, LN))
    wut = wu_v[...].astype(F32).T
    for k in range(R):
        wub[k] = jnp.broadcast_to(wut[:, k:k + 1], (C, LN))

    lax.fori_loop(NMAIN - NSEM, NMAIN, drain_step, (NMAIN - NSEM) % NB)

    wait_tail(0)
    (s0, r0, n0), = TAILS[0][1]
    assert r0 == 0 and n0 % RB == 0 and n0 >= RH
    add_blocks(s0, s0 % NB, n0 // RB)
    acc[...] = accb[...].reshape(NG, 3, 8, LN).sum(axis=1).reshape(C, LN)

    def pair_sum(hs, q):
        v = None
        for h in hs:
            parts = [buf[s, pl.ds(r, n)] for s, r, n in _split(h * RH + 48 * q, 48)]
            u = (parts[0] if len(parts) == 1 else jnp.concatenate(parts, axis=0)).astype(F32)
            v = u if v is None else v + u
        return jnp.concatenate(
            [v[0:8] + v[8:16] + v[16:24], v[24:32] + v[32:40] + v[40:48]], axis=0)

    n_early = 1 + len(TAIL_EARLY)
    for t in range(1, n_early):
        wait_tail(t)
        for q in range(CN // 16):
            acc[pl.ds(16 * q, 16)] += pair_sum(TAILS[t][0], q)

    sums = jnp.broadcast_to(jnp.sum(acc[pl.ds(0, CN)], axis=1, keepdims=True), (CN, LN))
    wdc[C - CN] = jnp.dot(wdt_v[:, pl.ds(0, CN)].astype(F32) * down_scale, sums,
                          preferred_element_type=F32, precision=lax.Precision.HIGHEST)
    late = acc[pl.ds(CN, C - CN)]
    for t in range(n_early, len(TAILS)):
        wait_tail(t)
        late = late + pair_sum(TAILS[t][0], CN // 16)
    late = jnp.broadcast_to(jnp.sum(late, axis=1, keepdims=True), (C - CN, LN))
    q1 = _tree_sum([wdc[C - CN]] + [wdc[c] * late[c:c + 1] for c in range(C - CN)])
    hid = q1 * _inv_1p_exp2(q1)
    hid = [jnp.broadcast_to(hid[k:k + 1], (8, LN)) for k in range(R)]

    gates = {}

    def gate(g):
        if g not in gates:
            q2 = _tree_sum([wub[k, pl.ds(8 * g, 8)] * hid[k] for k in range(R)])
            gates[g] = _inv_1p_exp2(q2)
        return gates[g]

    def rows(get, tile0, nrows):
        return jnp.concatenate([get((tile0 + i) // 3) for i in range(nrows // 8)], axis=0)

    def stripes(get, tile0, nrows):
        return jnp.stack([rows(get, tile0 + 8 * a, nrows) for a in range(A)])

    def emit(sl, scale):
        buf[sl] = (buf[sl].astype(F32) * scale).astype(buf.dtype)
        pltpu.make_async_copy(buf.at[sl], o_hbm.at[sl], sem_x).start()

    for a in range(A):
        emit((a, pl.ds(0, P0)), rows(gate, 8 * a, P0))
    for i in range(NSTATIC):
        emit((pl.ds(0, A), pl.ds(P0 + P * i, P)), stripes(gate, (P0 + P * i) // 8, P))
    for g in range(stab.shape[0]):
        stab[g] = gate(g % NG)

    def piece(s, i, u):
        tab = stab[pl.ds(u, NTAB)]
        r = pl.multiple_of(P0 + P * i, 16)
        emit((pl.ds(s, A), pl.ds(r, P)), stripes(lambda q: tab[q], 2, P))
        return jnp.where(u == NG - 2, 0, u + 2)

    def group(g, u0):
        tab = stab[pl.ds(u0, NTAB)]
        emit((pl.ds(A * g, A), pl.ds(0, P0)), stripes(lambda q: tab[q], 0, P0))
        lax.fori_loop(0, NP, lambda i, u: piece(A * g, i, u), u0 + 2)
        return jnp.where(u0 >= 8, u0 - 8, u0 + 16)

    lax.fori_loop(NSTATIC, NP, lambda i, u: piece(0, i, u), 2 + 2 * NSTATIC)
    lax.fori_loop(1, G, group, 16)


def _kernel(x_hbm, wdt_hbm, wu_hbm, o_hbm, buf, *scratch):
    def with_sem(sem_x):
        pl.run_scoped(
            lambda sem_in: _body(x_hbm, wdt_hbm, wu_hbm, o_hbm, buf, *scratch, sem_x, sem_in),
            pltpu.SemaphoreType.DMA((NSEM,)))
        pltpu.make_async_copy(buf, o_hbm, sem_x).wait()

    pl.run_scoped(with_sem, pltpu.SemaphoreType.DMA(()))


@jax.jit
def pallas_standalone__se_block__vision_kernel(
    x: jax.Array,
    w_down: jax.Array,
    w_up: jax.Array,
):
    assert x.shape == (1, H, W, C) and w_down.shape == (C, R) and w_up.shape == (R, C)
    xt = jnp.transpose(x, (0, 1, 3, 2)).reshape(H, NG, 8, W // LN, LN)
    xt = jnp.transpose(xt, (0, 1, 3, 2, 4)).reshape(NS, RS, LN)
    out = pl.pallas_call(
        _kernel,
        out_shape=jax.ShapeDtypeStruct((NS, RS, LN), x.dtype),
        in_specs=[pl.BlockSpec(memory_space=pl.ANY)] * 3,
        out_specs=pl.BlockSpec(memory_space=pl.ANY),
        scratch_shapes=[
            pltpu.VMEM((NS, RS, LN), x.dtype),
            pltpu.VMEM((NB, RB, LN), F32),
            pltpu.VMEM((C, LN), F32),
            pltpu.VMEM((NG + NTAB - 2, 8, LN), F32),
            pltpu.VMEM((R, C), w_down.dtype),
            pltpu.VMEM((R, C), w_up.dtype),
            pltpu.VMEM((C - CN + 1, R, LN), F32),
            pltpu.VMEM((R, C, LN), F32),
        ],
        compiler_params=pltpu.CompilerParams(vmem_limit_bytes=64 * 1024 * 1024),
    )(xt, w_down.T, w_up)
    out = out.reshape(H, NG, W // LN, 8, LN)
    out = jnp.transpose(out, (0, 1, 3, 2, 4)).reshape(1, H, C, W)
    return jnp.transpose(out, (0, 1, 3, 2))
```

```python
import jax
import jax.numpy as jnp
from jax import lax
import jax.experimental.pallas as pl
import jax.experimental.pallas.tpu as pltpu

F32 = jnp.float32
LOG2E = 1.4426950408889634

H, W, C, R = 384, 384, 192, 12
LN = 128
RH = C * W // LN
NG = C // 8
NS, RS = 54, 4096
RB = 64
NB = RH // RB

NSEM = 4
CN = C - 16
RC = 3 * CN
TAIL_EARLY = (8, 8, 4, 4)
TAIL_LATE = (18, 4, 2)

G, A = 9, 6
P0, P = 64, 48
NP = (RS - P0) // P
NSTATIC = 2
NTAB = 16


def _split(row0, nrows):
    out = []
    while nrows:
        s, r = divmod(row0, RS)
        n = min(nrows, RS - r)
        out.append((s, r, n))
        row0, nrows = row0 + n, nrows - n
    return out


def _plan_reads():
    h_tail = H - sum(TAIL_EARLY)
    nmain = h_tail * RH // RS
    groups = [((), _split(nmain * RS, h_tail * RH - nmain * RS))]
    for sizes, r0, nr in ((TAIL_EARLY, 0, RC), (TAIL_LATE, RC, RH - RC)):
        h0 = h_tail
        for n in sizes:
            hs = range(h0, h0 + n)
            groups.append((hs, [p for h in hs for p in _split(h * RH + r0, nr)]))
            h0 += n
        assert h0 == H
    return nmain, groups


NMAIN, TAILS = _plan_reads()


def _tree_sum(terms):
    while len(terms) > 1:
        terms = [terms[i] + terms[i + 1] if i + 1 < len(terms) else terms[i]
                 for i in range(0, len(terms), 2)]
    return terms[0]


def _clamp(q):
    return jnp.minimum(q, 120.0)


def _inv_1p_exp2(q):
    d = 1.0 + jnp.exp2(q)
    r = pl.reciprocal(d, approx=True)
    return r * (2.0 - d * r)


def _body(x_hbm, wdt_hbm, wu_hbm, o_hbm, buf, accb, acc, stab, wdt_v, wu_v, wdc, wub,
          sem_x, sem_in):
    def read(s):
        slot = s % NSEM if isinstance(s, int) else lax.rem(s, NSEM)
        return pltpu.make_async_copy(x_hbm.at[s], buf.at[s], sem_in.at[slot])

    def tail_copies(t):
        return [pltpu.make_async_copy(x_hbm.at[s, pl.ds(r, n)], buf.at[s, pl.ds(r, n)],
                                      sem_in.at[(NMAIN + t) % NSEM])
                for s, r, n in TAILS[t][1]]

    def start_tail(t):
        for cp in tail_copies(t):
            cp.start()

    def wait_tail(t):
        for cp in tail_copies(t):
            cp.wait()
        if t + NSEM < len(TAILS):
            start_tail(t + NSEM)

    read(0).start()
    w_copies = [pltpu.make_async_copy(wdt_hbm, wdt_v, sem_x),
                pltpu.make_async_copy(wu_hbm, wu_v, sem_x)]
    for cp in w_copies:
        cp.start()
    for s in range(1, NSEM):
        read(s).start()

    accb[...] = jnp.zeros(accb.shape, F32)

    def add_blocks(s, b0, nblocks):
        for k in range(NB):
            v = buf[s, pl.ds(RB * k, RB)].astype(F32)
            for j in range(k + NB, nblocks, NB):
                v = v + buf[s, pl.ds(RB * j, RB)].astype(F32)
            b = b0 + k
            b = b % NB if isinstance(b, int) else jnp.where(b >= NB, b - NB, b)
            accb[b] += v

    def main_step(s, b0):
        read(s).wait()
        read(s + NSEM).start()
        add_blocks(s, b0, RS // RB)
        return jnp.where(b0 == NB - 1, 0, b0 + 1)

    def drain_step(s, b0):
        read(s).wait()
        for t in range(NSEM):
            pl.when(s == NMAIN - NSEM + t)(lambda t=t: start_tail(t))
        add_blocks(s, b0, RS // RB)
        return jnp.where(b0 == NB - 1, 0, b0 + 1)

    lax.fori_loop(0, NMAIN - NSEM, main_step, 0)

    for cp in w_copies:
        cp.wait()
    down_scale = -LOG2E / (H * W)
    wdt = wdt_v[...].astype(F32) * down_scale
    for c in range(C - CN):
        wdc[c] = jnp.broadcast_to(wdt[:, CN + c:CN + c + 1], (R, LN))
    wut = wu_v[...].astype(F32).T
    for k in range(R):
        wub[k] = jnp.broadcast_to(wut[:, k:k + 1], (C, LN))

    lax.fori_loop(NMAIN - NSEM, NMAIN, drain_step, (NMAIN - NSEM) % NB)

    wait_tail(0)
    (s0, r0, n0), = TAILS[0][1]
    assert r0 == 0 and n0 % RB == 0 and n0 >= RH
    add_blocks(s0, s0 % NB, n0 // RB)
    acc[...] = accb[...].reshape(NG, 3, 8, LN).sum(axis=1).reshape(C, LN)

    def pair_sum(hs, q):
        v = None
        for h in hs:
            parts = [buf[s, pl.ds(r, n)] for s, r, n in _split(h * RH + 48 * q, 48)]
            u = (parts[0] if len(parts) == 1 else jnp.concatenate(parts, axis=0)).astype(F32)
            v = u if v is None else v + u
        return jnp.concatenate(
            [v[0:8] + v[8:16] + v[16:24], v[24:32] + v[32:40] + v[40:48]], axis=0)

    n_early = 1 + len(TAIL_EARLY)
    for t in range(1, n_early):
        wait_tail(t)
        for q in range(CN // 16):
            acc[pl.ds(16 * q, 16)] += pair_sum(TAILS[t][0], q)

    sums = jnp.broadcast_to(jnp.sum(acc[pl.ds(0, CN)], axis=1, keepdims=True), (CN, LN))
    wdc[C - CN] = jnp.dot(wdt_v[:, pl.ds(0, CN)].astype(F32) * down_scale, sums,
                          preferred_element_type=F32, precision=lax.Precision.HIGHEST)
    late = acc[pl.ds(CN, C - CN)]
    for t in range(n_early, len(TAILS)):
        wait_tail(t)
        late = late + pair_sum(TAILS[t][0], CN // 16)
    late = jnp.broadcast_to(jnp.sum(late, axis=1, keepdims=True), (C - CN, LN))
    q1 = _clamp(_tree_sum([wdc[C - CN]] + [wdc[c] * late[c:c + 1] for c in range(C - CN)]))
    hid = q1 * _inv_1p_exp2(q1)
    hid = [jnp.broadcast_to(hid[k:k + 1], (8, LN)) for k in range(R)]

    gates = {}

    def gate(g):
        if g not in gates:
            q2 = _tree_sum([wub[k, pl.ds(8 * g, 8)] * hid[k] for k in range(R)])
            gates[g] = _inv_1p_exp2(_clamp(q2))
        return gates[g]

    def rows(get, tile0, nrows):
        return jnp.concatenate([get((tile0 + i) // 3) for i in range(nrows // 8)], axis=0)

    def stripes(get, tile0, nrows):
        return jnp.stack([rows(get, tile0 + 8 * a, nrows) for a in range(A)])

    def emit(sl, scale):
        buf[sl] = (buf[sl].astype(F32) * scale).astype(buf.dtype)
        pltpu.make_async_copy(buf.at[sl], o_hbm.at[sl], sem_x).start()

    for a in range(A):
        emit((a, pl.ds(0, P0)), rows(gate, 8 * a, P0))
    for i in range(NSTATIC):
        emit((pl.ds(0, A), pl.ds(P0 + P * i, P)), stripes(gate, (P0 + P * i) // 8, P))
    for g in range(stab.shape[0]):
        stab[g] = gate(g % NG)

    def piece(s, i, u):
        tab = stab[pl.ds(u, NTAB)]
        r = pl.multiple_of(P0 + P * i, 16)
        emit((pl.ds(s, A), pl.ds(r, P)), stripes(lambda q: tab[q], 2, P))
        return jnp.where(u == NG - 2, 0, u + 2)

    def group(g, u0):
        tab = stab[pl.ds(u0, NTAB)]
        emit((pl.ds(A * g, A), pl.ds(0, P0)), stripes(lambda q: tab[q], 0, P0))
        lax.fori_loop(0, NP, lambda i, u: piece(A * g, i, u), u0 + 2)
        return jnp.where(u0 >= 8, u0 - 8, u0 + 16)

    lax.fori_loop(NSTATIC, NP, lambda i, u: piece(0, i, u), 2 + 2 * NSTATIC)
    lax.fori_loop(1, G, group, 16)


def _kernel(x_hbm, wdt_hbm, wu_hbm, o_hbm, buf, *scratch):
    def with_sem(sem_x):
        pl.run_scoped(
            lambda sem_in: _body(x_hbm, wdt_hbm, wu_hbm, o_hbm, buf, *scratch, sem_x, sem_in),
            pltpu.SemaphoreType.DMA((NSEM,)))
        pltpu.make_async_copy(buf, o_hbm, sem_x).wait()

    pl.run_scoped(with_sem, pltpu.SemaphoreType.DMA(()))


@jax.jit
def pallas_standalone__se_block__vision_kernel(
    x: jax.Array,
    w_down: jax.Array,
    w_up: jax.Array,
):
    assert x.shape == (1, H, W, C) and w_down.shape == (C, R) and w_up.shape == (R, C)
    xt = jnp.transpose(x, (0, 1, 3, 2)).reshape(H, NG, 8, W // LN, LN)
    xt = jnp.transpose(xt, (0, 1, 3, 2, 4)).reshape(NS, RS, LN)
    out = pl.pallas_call(
        _kernel,
        out_shape=jax.ShapeDtypeStruct((NS, RS, LN), x.dtype),
        in_specs=[pl.BlockSpec(memory_space=pl.ANY)] * 3,
        out_specs=pl.BlockSpec(memory_space=pl.ANY),
        scratch_shapes=[
            pltpu.VMEM((NS, RS, LN), x.dtype),
            pltpu.VMEM((NB, RB, LN), F32),
            pltpu.VMEM((C, LN), F32),
            pltpu.VMEM((NG + NTAB - 2, 8, LN), F32),
            pltpu.VMEM((R, C), w_down.dtype),
            pltpu.VMEM((R, C), w_up.dtype),
            pltpu.VMEM((C - CN + 1, R, LN), F32),
            pltpu.VMEM((R, C, LN), F32),
        ],
        compiler_params=pltpu.CompilerParams(vmem_limit_bytes=64 * 1024 * 1024),
    )(xt, w_down.T, w_up)
    out = out.reshape(H, NG, W // LN, 8, LN)
    out = jnp.transpose(out, (0, 1, 3, 2, 4)).reshape(1, H, C, W)
    return jnp.transpose(out, (0, 1, 3, 2))
```
